```python
import jax
import jax.numpy as jnp

def _softmax(x, axis=-1):
    return jax.nn.softmax(x, axis=axis)
def _gelu(x):
    return jax.nn.gelu(x, approximate=True)
def _silu(x):
    return jax.nn.silu(x)
def _sigmoid(x):
    return jax.nn.sigmoid(x)
def _layernorm(x, axis=-1, eps=1e-5):
    m = jnp.mean(x, axis=axis, keepdims=True)
    v = jnp.var(x, axis=axis, keepdims=True)
    return (x - m) / jnp.sqrt(v + eps)
def _scatter_add(tgt, idx, src, axis=0):
    return tgt.at[idx].add(src)
def _segment_sum(src, seg, n):
    return jax.ops.segment_sum(src, seg, n)
class _Rng:
    def __init__(self, key):
        self._k = key
    def _next(self):
        self._k, sub = jax.random.split(self._k)
        return sub
    def normal(self, shape):
        return jax.random.normal(self._next(), shape, dtype=jnp.bfloat16)
    def randint(self, lo, hi, shape):
        return jax.random.randint(self._next(), shape, lo, hi, dtype=jnp.int32)
    def uniform(self, shape, lo=0.0, hi=1.0):
        return jax.random.uniform(self._next(), shape, jnp.bfloat16, lo, hi)
    def permutation(self, n):
        return jax.random.permutation(self._next(), n)


kernel_name = 'recurrent_scan__sliding_block_cached__moe_arch_mod__prompt'

def setup_inputs():
    _rng = _Rng(jax.random.key(int.from_bytes(__import__("os").urandom(4), "little")))
    _w = (lambda a: (lambda t: t.astype(jnp.bfloat16) if jnp.issubdtype(t.dtype, jnp.floating) else t)(jnp.asarray(a)))
    def _A_setup():
        B, Sq, D = 1, 2048, 640
        Hq, Hkv, Sk, Dh = 32, 32, 2048, 192
        assert Hq % Hkv == 0, (Hq, Hkv)
        return {
            "x": _w((lambda *s: _rng.normal(s) * 0.05)(B, Sq, D)),
            "k_cache": _w((lambda *s: _rng.normal(s) * 0.05)(B, Hkv, Sk, Dh)),
            "v_cache": _w((lambda *s: _rng.normal(s) * 0.05)(B, Hkv, Sk, Dh)),
            "wq": _w((lambda *s: _rng.normal(s) * 0.05)(D, Hq * Dh) * (D ** -0.5)),
            "wo": _w((lambda *s: _rng.normal(s) * 0.05)(Hq * Dh, D) * ((Hq * Dh) ** -0.5)),
        }
    _A_in = _A_setup()

    def _B_setup():
        B, S, D, F, C = 1, 2048, 640, 1536, 2
        return {
            "x": _w((lambda *s: _rng.normal(s) * 0.05)(B, S, D)),
            "w_r": _w((lambda *s: _rng.normal(s) * 0.05)(D)),
            "w_gate": _w((lambda *s: _rng.normal(s) * 0.05)(D, F)),
            "w_up": _w((lambda *s: _rng.normal(s) * 0.05)(D, F)),
            "w_down": _w((lambda *s: _rng.normal(s) * 0.05)(F, D)),
        }
    _B_in = _B_setup()

    return {
        "A_x": _A_in["x"],
        "A_k_cache": _A_in["k_cache"],
        "A_v_cache": _A_in["v_cache"],
        "A_wq": _A_in["wq"],
        "A_wo": _A_in["wo"],
        "B_x": _B_in["x"],
        "B_w_r": _B_in["w_r"],
        "B_w_gate": _B_in["w_gate"],
        "B_w_up": _B_in["w_up"],
        "B_w_down": _B_in["w_down"],
    }

def reference(A_x, A_k_cache, A_v_cache, A_wq, A_wo, B_x, B_w_r, B_w_gate, B_w_up, B_w_down):
    def _A_ref(x, k_cache, v_cache, wq, wo):
        B, Sq, D = x.shape
        Hq, Dh = 32, 192
        Hkv, Sk = k_cache.shape[1], k_cache.shape[2]
        W = min(4096, max(256, Sk // 4))
        rep = Hq // Hkv
        q = (lambda x, *d: x.transpose(*d))((x @ wq).reshape(B, Sq, Hq, Dh), 0, 2, 1, 3)
        k = jnp.repeat(k_cache[:, :, Sk - W:, :], rep, axis=1)
        v = jnp.repeat(v_cache[:, :, Sk - W:, :], rep, axis=1)
        scores = jnp.einsum("bhqd,bhkd->bhqk", q, k) * (Dh ** -0.5)
        p = _softmax(scores, axis=-1)
        o = jnp.einsum("bhqk,bhkd->bhqd", p, v)
        return (lambda x, *d: x.transpose(*d))(o, 0, 2, 1, 3).reshape(B, Sq, Hq * Dh) @ wo

    def _B_ref(x, w_r, w_gate, w_up, w_down):
        B, S, D = x.shape
        C = 2
        r = x @ w_r
        idx = jnp.argsort(-r, axis=-1)[:, :C]
        idx_e = jnp.repeat(idx.reshape(B, C, 1), D, axis=2)
        x_sel = jnp.take_along_axis(x, idx_e, axis=1)
        g = _silu(x_sel @ w_gate)
        u = x_sel @ w_up
        y = (g * u) @ w_down
        r_sel = _sigmoid(jnp.take_along_axis(r, idx, axis=1))
        y = y * r_sel.reshape(B, C, 1)
        b_off = (jnp.arange(B) * S).reshape(B, 1)
        flat_idx = (idx + b_off).reshape(B * C)
        zero = (x * 0.0).reshape(B * S, D)
        upd = _scatter_add(zero, flat_idx, y.reshape(B * C, D), axis=0)
        return x + upd.reshape(B, S, D)

    x = A_x
    xn = _layernorm(x, axis=-1)
    s = _A_ref(xn, A_k_cache, A_v_cache, A_wq, A_wo)
    g = _silu(_B_ref(xn, B_w_r, B_w_gate, B_w_up, B_w_down))
    return x + s * g
```

```python
import functools
import jax, jax.numpy as jnp
from jax import lax
import jax.experimental.pallas as pl
import jax.experimental.pallas.tpu as pltpu

S, D, H, DH, W, F = 2048, 640, 32, 192, 512, 1536
LOG2E = 1.4426950408889634

def _build(bq=512, unroll=True, flags=None):
    nq = S // bq
    def kernel(x_ref, k_ref, v_ref, wq_ref, wo_ref, wr_ref, wg_ref, wu_ref, wd_ref, o_ref,
               xn_ref, acc_ref, kp_ref, vp_ref):
        j = pl.program_id(0)
        nj = pl.num_programs(0)

        @pl.when(j == 0)
        def _():
            def ln(i, c):
                r0 = pl.multiple_of(i * 128, 128)
                x = x_ref[pl.ds(r0, 128), :].astype(jnp.float32)
                m = jnp.mean(x, axis=-1, keepdims=True)
                xc = x - m
                v = jnp.mean(xc * xc, axis=-1, keepdims=True)
                xn_ref[pl.ds(r0, 128), :] = (xc * lax.rsqrt(v + 1e-5)).astype(jnp.bfloat16)
                acc_ref[pl.ds(r0, 128), :] = jnp.zeros((128, D), jnp.float32)
                return c
            lax.fori_loop(0, S // 128, ln, 0)

        z64 = jnp.zeros((64, W), jnp.bfloat16)
        kp_ref[0, 0:192] = k_ref[0]
        kp_ref[0, 192:256] = z64
        kp_ref[1, 0:64] = z64
        kp_ref[1, 64:256] = k_ref[1]
        vp_ref[0, 0:192] = v_ref[0]
        vp_ref[0, 192:256] = z64
        vp_ref[1, 0:64] = z64
        vp_ref[1, 64:256] = v_ref[1]

        def body(i, c):
            r0 = pl.multiple_of(i * bq, bq)
            xn = xn_ref[pl.ds(r0, bq), :]
            q = jnp.dot(xn, wq_ref[...], preferred_element_type=jnp.float32)
            q = (q * (DH ** -0.5 * LOG2E)).astype(jnp.bfloat16)
            os_ = []
            for h in range(2):
                qh = q[:, h * 128:h * 128 + 256]
                s = jnp.dot(qh, kp_ref[h], preferred_element_type=jnp.float32)
                m = jnp.max(s, axis=-1, keepdims=True)
                p = jnp.exp2(s - m)
                l = jnp.sum(p, axis=-1, keepdims=True)
                o = lax.dot_general(p.astype(jnp.bfloat16), vp_ref[h], (((1,), (1,)), ((), ())), preferred_element_type=jnp.float32)
                os_.append(o * (1.0 / l))
            oc = jnp.concatenate([os_[0][:, :128], os_[0][:, 128:] + os_[1][:, :128], os_[1][:, 128:]], axis=1)
            acc_ref[pl.ds(r0, bq), :] += jnp.dot(oc.astype(jnp.bfloat16), wo_ref[...], preferred_element_type=jnp.float32)
            return c
        if unroll:
            for i in range(nq):
                body(i, 0)
        else:
            lax.fori_loop(0, nq, body, 0)

        @pl.when(j == nj - 1)
        def _():
            xn = xn_ref[...]
            wr = wr_ref[...]
            r = lax.dot_general(wr, xn, (((1,), (1,)), ((), ())), preferred_element_type=jnp.float32)
            r = r[0:1, :]
            lane = lax.broadcasted_iota(jnp.int32, (1, S), 1)
            m1 = jnp.max(r, axis=-1, keepdims=True)
            i1 = jnp.min(jnp.where(r == m1, lane, S), axis=-1, keepdims=True)
            r2 = jnp.where(lane == i1, -jnp.inf, r)
            m2 = jnp.max(r2, axis=-1, keepdims=True)
            i2 = jnp.min(jnp.where((r2 == m2) & (lane != i1), lane, S), axis=-1, keepdims=True)
            row8 = lax.broadcasted_iota(jnp.int32, (8, S), 0)
            lane8 = lax.broadcasted_iota(jnp.int32, (8, S), 1)
            sel = jnp.where(((row8 == 0) & (lane8 == i1)) | ((row8 == 1) & (lane8 == i2)), 1.0, 0.0).astype(jnp.bfloat16)
            xs = jnp.dot(sel, xn, preferred_element_type=jnp.float32).astype(jnp.bfloat16)
            g = jnp.dot(xs, wg_ref[...], preferred_element_type=jnp.float32)
            u = jnp.dot(xs, wu_ref[...], preferred_element_type=jnp.float32)
            hgu = (g * jax.nn.sigmoid(g) * u).astype(jnp.bfloat16)
            y = jnp.dot(hgu, wd_ref[...], preferred_element_type=jnp.float32)
            y1 = y[0:1, :] * jax.nn.sigmoid(m1)
            y2 = y[1:2, :] * jax.nn.sigmoid(m2)
            def fin(i, c):
                r0 = pl.multiple_of(i * 128, 128)
                rows = lax.broadcasted_iota(jnp.int32, (128, 1), 0) + r0
                b = xn_ref[pl.ds(r0, 128), :].astype(jnp.float32)
                b = b + jnp.where(rows == i1, y1, 0.0) + jnp.where(rows == i2, y2, 0.0)
                gg = b * jax.nn.sigmoid(b)
                o_ref[pl.ds(r0, 128), :] = (x_ref[pl.ds(r0, 128), :].astype(jnp.float32) + acc_ref[pl.ds(r0, 128), :] * gg).astype(o_ref.dtype)
                return c
            lax.fori_loop(0, S // 128, fin, 0)

    def fn(A_x, A_k_cache, A_v_cache, A_wq, A_wo, B_x, B_w_r, B_w_gate, B_w_up, B_w_down):
        x = A_x.reshape(S, D)
        k = A_k_cache.reshape(H, 2048, DH).transpose(0, 2, 1)
        v = A_v_cache.reshape(H, 2048, DH).transpose(0, 2, 1)
        wr = jnp.broadcast_to(B_w_r.reshape(1, D), (8, D))
        c = lambda j: (0, 0)
        out = pl.pallas_call(
            kernel,
            grid=(H // 2,),
            in_specs=[
                pl.BlockSpec((S, D), c),
                pl.BlockSpec((2, DH, W), lambda j: (j, 0, 3)),
                pl.BlockSpec((2, DH, W), lambda j: (j, 0, 3)),
                pl.BlockSpec((D, 2 * DH), lambda j: (0, j)),
                pl.BlockSpec((2 * DH, D), lambda j: (j, 0)),
                pl.BlockSpec((8, D), c),
                pl.BlockSpec((D, F), c),
                pl.BlockSpec((D, F), c),
                pl.BlockSpec((F, D), c),
            ],
            out_specs=pl.BlockSpec((S, D), c),
            out_shape=jax.ShapeDtypeStruct((S, D), jnp.bfloat16),
            scratch_shapes=[
                pltpu.VMEM((S, D), jnp.bfloat16),
                pltpu.VMEM((S, D), jnp.float32),
                pltpu.VMEM((2, 256, W), jnp.bfloat16),
                pltpu.VMEM((2, 256, W), jnp.bfloat16),
            ],
            compiler_params=pltpu.CompilerParams(
                dimension_semantics=("arbitrary",), vmem_limit_bytes=100 * 1024 * 1024,
                **({"flags": flags} if flags else {})),
        )(x, k, v, A_wq, A_wo, wr, B_w_gate, B_w_up, B_w_down)
        return out.reshape(1, S, D)
    return fn


@jax.jit
def pallas_recurrent_scan__sliding_block_cached__moe_arch_mod__prompt_kernel(
    A_x, A_k_cache, A_v_cache, A_wq, A_wo, B_x, B_w_r, B_w_gate, B_w_up, B_w_down):
    return _build()(A_x, A_k_cache, A_v_cache, A_wq, A_wo, B_x, B_w_r, B_w_gate, B_w_up, B_w_down)
```

```python
import functools, contextlib
import jax, jax.numpy as jnp
from jax import lax
import jax.experimental.pallas as pl
import jax.experimental.pallas.tpu as pltpu

S, D, H, DH, W, F = 2048, 640, 32, 192, 512, 1536
LOG2E = 1.4426950408889634
NT = (((1,), (1,)), ((), ()))
f32, bf16 = jnp.float32, jnp.bfloat16

def _build(bq=2048, flags=None, lnb=256, lnu=1, nxc=8, finb=128, finu=2, noc=8, scopes=False, ffn_step=1,
         nosm=False, mode='H1', gsteps=8, FC=512, gpos=1, usetanh=True):
    nq = S // bq
    NP = H // 2
    sc = (lambda n: jax.named_scope(n)) if scopes else (lambda n: contextlib.nullcontext())
    xc_rows = S // nxc
    oc_rows = S // noc
    gb = S // gsteps
    std_acc = mode == 'H2'

    def kernel(x_hbm, k_hbm, v_hbm, wq_hbm, wo_hbm, wr_hbm, wg_hbm, wu_hbm, wd_hbm, o_hbm,
               x_ref, xn_ref, g_ref, ix_ref, acc_ref, kp_ref, wot_ref,
               wg_ref, wu_ref, wd_ref, ob_ref, r_ref, kb_ref, vb_ref, wqb_ref, wob_ref, wr_ref, xsem, wsem, osem, psem, rsem):
        j = pl.program_id(0)
        slot = j % 2

        def pcopies(p, s):
            h0 = p * 2
            c0 = pl.multiple_of(p * (2 * DH), 2 * DH)
            return [pltpu.make_async_copy(k_hbm.at[pl.ds(h0, 2), :, pl.ds(3 * W, W)], kb_ref.at[s], psem.at[s, 0]),
                    pltpu.make_async_copy(v_hbm.at[pl.ds(h0, 2), :, pl.ds(3 * W, W)], vb_ref.at[s], psem.at[s, 1]),
                    pltpu.make_async_copy(wq_hbm.at[:, pl.ds(c0, 2 * DH)], wqb_ref.at[s], psem.at[s, 2]),
                    pltpu.make_async_copy(wo_hbm.at[pl.ds(c0, 2 * DH), :], wob_ref.at[s], psem.at[s, 3])]

        def xcopy(c):
            r0 = pl.multiple_of(c * xc_rows, xc_rows)
            return pltpu.make_async_copy(x_hbm.at[pl.ds(r0, xc_rows)], x_ref.at[pl.ds(r0, xc_rows)], xsem.at[c])
        def wcopies():
            return [pltpu.make_async_copy(wg_hbm, wg_ref, wsem.at[0]),
                    pltpu.make_async_copy(wu_hbm, wu_ref, wsem.at[1]),
                    pltpu.make_async_copy(wd_hbm, wd_ref, wsem.at[2])]
        def ocopy(c):
            r0 = pl.multiple_of(c * oc_rows, oc_rows)
            return pltpu.make_async_copy(ob_ref.at[pl.ds(r0, oc_rows)], o_hbm.at[pl.ds(r0, oc_rows)], osem.at[c])

        def _first():
            rcopy = pltpu.make_async_copy(wr_hbm, wr_ref, rsem)
            rcopy.start()
            for c in range(nxc):
                xcopy(c).start()
            for cp in pcopies(0, 0):
                cp.start()
            acc_ref[...] = jnp.zeros_like(acc_ref)
            rcopy.wait()
            wr = wr_ref[...]
            def chunk(c, carry):
                xcopy(c).wait()
                def ln(b, carry2):
                    for u in range(lnu):
                        r0 = pl.multiple_of(c * xc_rows + (b * lnu + u) * lnb, lnb)
                        x = x_ref[pl.ds(r0, lnb), :].astype(f32)
                        m = jnp.mean(x, axis=-1, keepdims=True)
                        xc = x - m
                        v = jnp.mean(xc * xc, axis=-1, keepdims=True)
                        xn = (xc * lax.rsqrt(v + 1e-5)).astype(bf16)
                        xn_ref[pl.ds(r0, lnb), :] = xn
                        if lnb >= 128:
                            r_ref[:, pl.ds(r0, lnb)] = lax.dot_general(wr, xn, NT, preferred_element_type=f32)
                    return carry2
                lax.fori_loop(0, xc_rows // (lnb * lnu), ln, 0)
                return carry
            lax.fori_loop(0, nxc, chunk, 0)
            for cp in wcopies():
                cp.start()
        with sc("LN"):
            pl.when(j == 0)(_first)

        def _ffn():
            for cp in wcopies():
                cp.wait()
            xn = xn_ref[...]
            if lnb >= 128:
                r = r_ref[0:1, :]
            else:
                r = lax.dot_general(wr_ref[...], xn, NT, preferred_element_type=f32)[0:1, :]
            lane = lax.broadcasted_iota(jnp.int32, (1, S), 1)
            m1 = jnp.max(r, axis=-1, keepdims=True)
            i1 = jnp.min(jnp.where(r == m1, lane, S), axis=-1, keepdims=True)
            r2 = jnp.where(lane == i1, -jnp.inf, r)
            m2 = jnp.max(r2, axis=-1, keepdims=True)
            i2 = jnp.min(jnp.where((r2 == m2) & (lane != i1), lane, S), axis=-1, keepdims=True)
            row8 = lax.broadcasted_iota(jnp.int32, (8, S), 0)
            lane8 = lax.broadcasted_iota(jnp.int32, (8, S), 1)
            sel = jnp.where(((row8 == 0) & (lane8 == i1)) | ((row8 == 1) & (lane8 == i2)), 1.0, 0.0).astype(bf16)
            xs = jnp.dot(sel, xn, preferred_element_type=f32)
            xsb = xs.astype(bf16)
            y = jnp.zeros((8, D), f32)
            def fch(c, y):
                c0 = pl.multiple_of(c * FC, FC)
                gt = jnp.dot(xsb, wg_ref[:, pl.ds(c0, FC)], preferred_element_type=f32)
                u = jnp.dot(xsb, wu_ref[:, pl.ds(c0, FC)], preferred_element_type=f32)
                hgu = (gt * jax.nn.sigmoid(gt) * u).astype(bf16)
                return y + jnp.dot(hgu, wd_ref[pl.ds(c0, FC), :], preferred_element_type=f32)
            y = lax.fori_loop(0, F // FC, fch, y)
            mm = jnp.where(lax.broadcasted_iota(jnp.int32, (8, 1), 0) == 0, m1, m2)
            b = xs + y * jax.nn.sigmoid(mm)
            gp = b * jax.nn.sigmoid(b)
            g_ref[...] = gp
            ix_ref[...] = jnp.broadcast_to(jnp.where(lax.broadcasted_iota(jnp.int32, (8, 1), 0) == 0, i1, i2), (8, 128))
        with sc("FFN"):
            pl.when(j == ffn_step)(_ffn)

        @pl.when(j + 1 < NP)
        def _():
            for cp in pcopies(j + 1, 1 - slot):
                cp.start()
        for cp in pcopies(j, slot):
            cp.wait()
        k_ref, v_ref, wq_ref, wo_ref = kb_ref.at[slot], vb_ref.at[slot], wqb_ref.at[slot], wob_ref.at[slot]

        with sc("MAIN"):
            def prep():
                z64 = jnp.zeros((64, W), bf16)
                kp_ref[0] = jnp.concatenate([k_ref[0], z64], axis=0).T
                kp_ref[1] = jnp.concatenate([z64, k_ref[1]], axis=0).T
            def prep_wo():
                if not std_acc:
                    wot_ref[...] = wo_ref[...].T
            def gate(part, nparts):
                rows = gb // nparts
                g0 = pl.multiple_of(jnp.minimum(j, gsteps) * gb + part * rows, rows)
                g1 = pl.multiple_of(jnp.minimum(j, gsteps - 1) * gb + part * rows, rows)
                b = xn_ref[pl.ds(g1, rows), :].astype(f32)
                g_ref[pl.ds(g0, rows), :] = b * jax.nn.sigmoid(b)
            for i in range(nq):
                r0 = i * bq
                q = jnp.dot(xn_ref[r0:r0 + bq, :], wq_ref[...], preferred_element_type=f32)
                q = (q * (DH ** -0.5 * LOG2E)).astype(bf16)
                if i == 0:
                    prep()
                os_ = []
                for h in range(2):
                    st = lax.dot_general(kp_ref[h], q[:, h * 128:h * 128 + 256], NT, preferred_element_type=f32)
                    if h == 0 and i == 0:
                        prep_wo()
                    if nosm:
                        o = jnp.dot(v_ref[h], st.astype(bf16), preferred_element_type=f32)
                        os_.append(o.astype(bf16))
                        continue
                    m = jnp.max(st, axis=0, keepdims=True)
                    p = jnp.exp2(st - m)
                    l = jnp.sum(p, axis=0, keepdims=True)
                    o = jnp.dot(v_ref[h], p.astype(bf16), preferred_element_type=f32)
                    os_.append((o * (1.0 / l)).astype(bf16))
                oc = jnp.concatenate(os_, axis=0)
                if not std_acc:
                    acc_ref[:, r0:r0 + bq] += jnp.dot(wot_ref[...], oc, preferred_element_type=f32)
                else:
                    acc_ref[r0:r0 + bq, :] += jnp.dot(oc.T, wo_ref[...], preferred_element_type=f32)

        def _fin():
            i1 = ix_ref[0:1, 0:1]
            i2 = ix_ref[1:2, 0:1]
            gp1 = g_ref[0:1, :]
            gp2 = g_ref[1:2, :]
            def chunk(c, carry):
                def fin(b, carry2):
                    for u in range(finu):
                        r0 = pl.multiple_of(c * oc_rows + (b * finu + u) * finb, finb)
                        bb = xn_ref[pl.ds(r0, finb), :].astype(f32)
                        gg = bb * (0.5 + 0.5 * jnp.tanh(0.5 * bb)) if usetanh else bb * jax.nn.sigmoid(bb)
                        rows = lax.broadcasted_iota(jnp.int32, (finb, 1), 0) + r0
                        gg = jnp.where(rows == i1, gp1, jnp.where(rows == i2, gp2, gg))
                        a = acc_ref[pl.ds(r0, finb), :] if std_acc else acc_ref[:, pl.ds(r0, finb)].T
                        ob_ref[pl.ds(r0, finb), :] = (x_ref[pl.ds(r0, finb), :].astype(f32) + a * gg).astype(bf16)
                    return carry2
                lax.fori_loop(0, oc_rows // (finb * finu), fin, 0)
                ocopy(c).start()
                return carry
            lax.fori_loop(0, noc, chunk, 0)
            for c in range(noc):
                ocopy(c).wait()
        with sc("FIN"):
            pl.when(j == NP - 1)(_fin)

    def fn(A_x, A_k_cache, A_v_cache, A_wq, A_wo, B_x, B_w_r, B_w_gate, B_w_up, B_w_down):
        x = A_x.reshape(S, D)
        k = A_k_cache.reshape(H, 2048, DH).transpose(0, 2, 1)
        v = A_v_cache.reshape(H, 2048, DH).transpose(0, 2, 1)
        wr = jnp.broadcast_to(B_w_r.reshape(1, D), (8, D))
        c = lambda j: (0, 0)
        anyspec = pl.BlockSpec(memory_space=pl.ANY)
        out = pl.pallas_call(
            kernel,
            grid=(NP,),
            in_specs=[
                anyspec] * 9 + [
            ],
            out_specs=anyspec,
            out_shape=jax.ShapeDtypeStruct((S, D), bf16),
            scratch_shapes=[
                pltpu.VMEM((S, D), bf16),
                pltpu.VMEM((S, D), bf16),
                pltpu.VMEM((8, D), f32),
                pltpu.VMEM((8, 128), jnp.int32),
                pltpu.VMEM((S, D) if std_acc else (D, S), f32),
                pltpu.VMEM((2, W, 256), bf16),
                pltpu.VMEM((D, 2 * DH), bf16),
                pltpu.VMEM((D, F), bf16),
                pltpu.VMEM((D, F), bf16),
                pltpu.VMEM((F, D), bf16),
                pltpu.VMEM((S, D), bf16),
                pltpu.VMEM((8, S), f32),
                pltpu.VMEM((2, 2, DH, W), bf16),
                pltpu.VMEM((2, 2, DH, W), bf16),
                pltpu.VMEM((2, D, 2 * DH), bf16),
                pltpu.VMEM((2, 2 * DH, D), bf16),
                pltpu.VMEM((8, D), bf16),
                pltpu.SemaphoreType.DMA((nxc,)),
                pltpu.SemaphoreType.DMA((3,)),
                pltpu.SemaphoreType.DMA((noc,)),
                pltpu.SemaphoreType.DMA((2, 4)),
                pltpu.SemaphoreType.DMA(()),
            ],
            compiler_params=pltpu.CompilerParams(
                dimension_semantics=("arbitrary",), vmem_limit_bytes=100 * 1024 * 1024,
                **({"flags": flags} if flags else {})),
        )(x, k, v, A_wq, A_wo, wr, B_w_gate, B_w_up, B_w_down)
        return out.reshape(1, S, D)
    return fn


@jax.jit
def pallas_recurrent_scan__sliding_block_cached__moe_arch_mod__prompt_kernel(
        A_x, A_k_cache, A_v_cache, A_wq, A_wo, B_x, B_w_r, B_w_gate, B_w_up, B_w_down):
    return _build()(A_x, A_k_cache, A_v_cache, A_wq, A_wo, B_x, B_w_r, B_w_gate, B_w_up, B_w_down)
```

```python
import functools, contextlib
import jax, jax.numpy as jnp
from jax import lax
import jax.experimental.pallas as pl
import jax.experimental.pallas.tpu as pltpu

S, D, H, DH, W, F = 2048, 640, 32, 192, 512, 1536
LOG2E = 1.4426950408889634
NT = (((1,), (1,)), ((), ()))
f32, bf16 = jnp.float32, jnp.bfloat16

def _build(bq=2048, flags=None, lnb=256, lnu=1, nxc=8, finb=128, finu=2, noc=8, scopes=False, ffn_step=1,
         nosm=False, mode='H1', gsteps=8, FC=512, gpos=1, usetanh=True, tb16=True, smode=0, cw=512, order=0, dmapos=0):
    nq = S // bq
    NP = H // 2
    sc = (lambda n: jax.named_scope(n)) if scopes else (lambda n: contextlib.nullcontext())
    xc_rows = S // nxc
    oc_rows = S // noc
    gb = S // gsteps
    std_acc = mode == 'H2'

    def kernel(x_hbm, k_hbm, v_hbm, wq_hbm, wo_hbm, wr_hbm, wg_hbm, wu_hbm, wd_hbm, o_hbm,
               x_ref, xn_ref, g_ref, acc_ref, kp_ref, wot_ref,
               wg_ref, wu_ref, wd_ref, ob_ref, r_ref, kb_ref, vb_ref, wqb_ref, wob_ref, wr_ref, p_ref, xsem, wsem, osem, psem, rsem):
        j = pl.program_id(0)
        slot = j % 2

        def pcopies(p, s):
            h0 = p * 2
            c0 = pl.multiple_of(p * (2 * DH), 2 * DH)
            return [pltpu.make_async_copy(k_hbm.at[pl.ds(h0, 2), :, pl.ds(3 * W, W)], kb_ref.at[s], psem.at[s, 0]),
                    pltpu.make_async_copy(v_hbm.at[pl.ds(h0, 2), :, pl.ds(3 * W, W)], vb_ref.at[s], psem.at[s, 1]),
                    pltpu.make_async_copy(wq_hbm.at[:, pl.ds(c0, 2 * DH)], wqb_ref.at[s], psem.at[s, 2]),
                    pltpu.make_async_copy(wo_hbm.at[pl.ds(c0, 2 * DH), :], wob_ref.at[s], psem.at[s, 3])]

        def xcopy(c):
            r0 = pl.multiple_of(c * xc_rows, xc_rows)
            return pltpu.make_async_copy(x_hbm.at[pl.ds(r0, xc_rows)], x_ref.at[pl.ds(r0, xc_rows)], xsem.at[c])
        def wcopies():
            return [pltpu.make_async_copy(wg_hbm, wg_ref, wsem.at[0]),
                    pltpu.make_async_copy(wu_hbm, wu_ref, wsem.at[1]),
                    pltpu.make_async_copy(wd_hbm, wd_ref, wsem.at[2])]
        def ocopy(c):
            r0 = pl.multiple_of(c * oc_rows, oc_rows)
            return pltpu.make_async_copy(ob_ref.at[pl.ds(r0, oc_rows)], o_hbm.at[pl.ds(r0, oc_rows)], osem.at[c])

        def _first():
            rcopy = pltpu.make_async_copy(wr_hbm, wr_ref, rsem)
            rcopy.start()
            for c in range(nxc):
                xcopy(c).start()
            for cp in pcopies(0, 0):
                cp.start()
            acc_ref[...] = jnp.zeros_like(acc_ref)
            rcopy.wait()
            wr = wr_ref[...]
            def chunk(c, carry):
                xcopy(c).wait()
                def ln(b, carry2):
                    for u in range(lnu):
                        r0 = pl.multiple_of(c * xc_rows + (b * lnu + u) * lnb, lnb)
                        x = x_ref[pl.ds(r0, lnb), :].astype(f32)
                        m = jnp.mean(x, axis=-1, keepdims=True)
                        xc = x - m
                        v = jnp.mean(xc * xc, axis=-1, keepdims=True)
                        xf = xc * lax.rsqrt(v + 1e-5)
                        xn = xf.astype(bf16)
                        xn_ref[pl.ds(r0, lnb), :] = xn
                        g_ref[pl.ds(r0, lnb), :] = xf * (0.5 + 0.5 * jnp.tanh(0.5 * xf))
                        if lnb >= 128:
                            r_ref[:, pl.ds(r0, lnb)] = lax.dot_general(wr, xn, NT, preferred_element_type=f32)
                    return carry2
                lax.fori_loop(0, xc_rows // (lnb * lnu), ln, 0)
                return carry
            lax.fori_loop(0, nxc, chunk, 0)
            for cp in wcopies():
                cp.start()
        with sc("LN"):
            pl.when(j == 0)(_first)

        def _ffn():
            for cp in wcopies():
                cp.wait()
            xn = xn_ref[...]
            if lnb >= 128:
                r = r_ref[0:1, :]
            else:
                r = lax.dot_general(wr_ref[...], xn, NT, preferred_element_type=f32)[0:1, :]
            lane = lax.broadcasted_iota(jnp.int32, (1, S), 1)
            m1 = jnp.max(r, axis=-1, keepdims=True)
            i1 = jnp.min(jnp.where(r == m1, lane, S), axis=-1, keepdims=True)
            r2 = jnp.where(lane == i1, -jnp.inf, r)
            m2 = jnp.max(r2, axis=-1, keepdims=True)
            i2 = jnp.min(jnp.where((r2 == m2) & (lane != i1), lane, S), axis=-1, keepdims=True)
            row8 = lax.broadcasted_iota(jnp.int32, (8, S), 0)
            lane8 = lax.broadcasted_iota(jnp.int32, (8, S), 1)
            sel = jnp.where(((row8 == 0) & (lane8 == i1)) | ((row8 == 1) & (lane8 == i2)), 1.0, 0.0).astype(bf16)
            xs = jnp.dot(sel, xn, preferred_element_type=f32)
            xsb = xs.astype(bf16)
            y = jnp.zeros((8, D), f32)
            def fch(c, y):
                c0 = pl.multiple_of(c * FC, FC)
                gt = jnp.dot(xsb, wg_ref[:, pl.ds(c0, FC)], preferred_element_type=f32)
                u = jnp.dot(xsb, wu_ref[:, pl.ds(c0, FC)], preferred_element_type=f32)
                hgu = (gt * jax.nn.sigmoid(gt) * u).astype(bf16)
                return y + jnp.dot(hgu, wd_ref[pl.ds(c0, FC), :], preferred_element_type=f32)
            y = lax.fori_loop(0, F // FC, fch, y)
            mm = jnp.where(lax.broadcasted_iota(jnp.int32, (8, 1), 0) == 0, m1, m2)
            b = xs + y * jax.nn.sigmoid(mm)
            gp = b * jax.nn.sigmoid(b)
            s1 = jnp.sum(i1)
            s2 = jnp.sum(i2)
            g_ref[pl.ds(s1, 1), :] = gp[0:1, :]
            g_ref[pl.ds(s2, 1), :] = gp[1:2, :]
        with sc("FFN"):
            pl.when(j == ffn_step)(_ffn)

        if dmapos == 0:
            @pl.when(j + 1 < NP)
            def _():
                for cp in pcopies(j + 1, 1 - slot):
                    cp.start()
        for cp in pcopies(j, slot):
            cp.wait()
        k_ref, v_ref, wq_ref, wo_ref = kb_ref.at[slot], vb_ref.at[slot], wqb_ref.at[slot], wob_ref.at[slot]

        with sc("MAIN"):
            def prep():
                z64 = jnp.zeros((64, W), bf16)
                kp_ref[0] = jnp.concatenate([k_ref[0], z64], axis=0).T
                kp_ref[1] = jnp.concatenate([z64, k_ref[1]], axis=0).T
            def prep_wo():
                if not std_acc:
                    wot_ref[...] = wo_ref[...].T
            def gate(part, nparts):
                rows = gb // nparts
                g0 = pl.multiple_of(jnp.minimum(j, gsteps) * gb + part * rows, rows)
                g1 = pl.multiple_of(jnp.minimum(j, gsteps - 1) * gb + part * rows, rows)
                b = xn_ref[pl.ds(g1, rows), :].astype(f32)
                g_ref[pl.ds(g0, rows), :] = b * jax.nn.sigmoid(b)
            for i in range(nq):
                r0 = i * bq
                q = jnp.dot(xn_ref[r0:r0 + bq, :], wq_ref[...], preferred_element_type=f32)
                q = (q * (DH ** -0.5 * LOG2E)).astype(bf16)
                if i == 0:
                    prep()
                os_ = []
                if dmapos == 1:
                    for cp in pcopies(jnp.minimum(j + 1, NP - 1), 1 - slot):
                        cp.start()
                def sdot(h):
                    return lax.dot_general(kp_ref[h], q[:, h * 128:h * 128 + 256], NT, preferred_element_type=f32)
                def smpv(h, st):
                    m = jnp.max(st, axis=0, keepdims=True)
                    p = jnp.exp2(st - m)
                    l = jnp.sum(p, axis=0, keepdims=True)
                    o = jnp.dot(v_ref[h], p.astype(bf16), preferred_element_type=f32)
                    return (o * (1.0 / l)).astype(bf16)
                if order == 0:
                    s0 = sdot(0); prep_wo(); o0 = smpv(0, s0); s1 = sdot(1); o1 = smpv(1, s1)
                elif order == 1:
                    s0 = sdot(0); s1 = sdot(1); prep_wo(); o0 = smpv(0, s0); o1 = smpv(1, s1)
                elif order == 2:
                    s0 = sdot(0); s1 = sdot(1); o0 = smpv(0, s0); prep_wo(); o1 = smpv(1, s1)
                elif order == 3:
                    s0 = sdot(0); o0 = smpv(0, s0); s1 = sdot(1); o1 = smpv(1, s1); prep_wo()
                os_ = [o0, o1]
                oc = jnp.concatenate(os_, axis=0)
                if not std_acc:
                    acc_ref[:, r0:r0 + bq] += jnp.dot(wot_ref[...], oc, preferred_element_type=f32)
                else:
                    acc_ref[r0:r0 + bq, :] += jnp.dot(oc.T, wo_ref[...], preferred_element_type=f32)

        def _fin():
            def chunk(c, carry):
                def fin(b, carry2):
                    for u in range(finu):
                        r0 = pl.multiple_of(c * oc_rows + (b * finu + u) * finb, finb)
                        gg = g_ref[pl.ds(r0, finb), :]
                        a = acc_ref[pl.ds(r0, finb), :] if std_acc else (acc_ref[:, pl.ds(r0, finb)].astype(bf16).T.astype(f32) if tb16 else acc_ref[:, pl.ds(r0, finb)].T)
                        ob_ref[pl.ds(r0, finb), :] = (x_ref[pl.ds(r0, finb), :].astype(f32) + a * gg).astype(bf16)
                    return carry2
                lax.fori_loop(0, oc_rows // (finb * finu), fin, 0)
                ocopy(c).start()
                return carry
            lax.fori_loop(0, noc, chunk, 0)
            for c in range(noc):
                ocopy(c).wait()
            if dmapos == 1:
                for cp in pcopies(NP - 1, 1 - slot):
                    cp.wait()
        with sc("FIN"):
            pl.when(j == NP - 1)(_fin)

    def fn(A_x, A_k_cache, A_v_cache, A_wq, A_wo, B_x, B_w_r, B_w_gate, B_w_up, B_w_down):
        x = A_x.reshape(S, D)
        k = A_k_cache.reshape(H, 2048, DH).transpose(0, 2, 1)
        v = A_v_cache.reshape(H, 2048, DH).transpose(0, 2, 1)
        wr = jnp.broadcast_to(B_w_r.reshape(1, D), (8, D))
        c = lambda j: (0, 0)
        anyspec = pl.BlockSpec(memory_space=pl.ANY)
        out = pl.pallas_call(
            kernel,
            grid=(NP,),
            in_specs=[
                anyspec] * 9 + [
            ],
            out_specs=anyspec,
            out_shape=jax.ShapeDtypeStruct((S, D), bf16),
            scratch_shapes=[
                pltpu.VMEM((S, D), bf16),
                pltpu.VMEM((S, D), bf16),
                pltpu.VMEM((S, D), f32),
                pltpu.VMEM((S, D) if std_acc else (D, S), f32),
                pltpu.VMEM((2, W, 256), bf16),
                pltpu.VMEM((D, 2 * DH), bf16),
                pltpu.VMEM((D, F), bf16),
                pltpu.VMEM((D, F), bf16),
                pltpu.VMEM((F, D), bf16),
                pltpu.VMEM((S, D), bf16),
                pltpu.VMEM((8, S), f32),
                pltpu.VMEM((2, 2, DH, W), bf16),
                pltpu.VMEM((2, 2, DH, W), bf16),
                pltpu.VMEM((2, D, 2 * DH), bf16),
                pltpu.VMEM((2, 2 * DH, D), bf16),
                pltpu.VMEM((8, D), bf16),
                pltpu.VMEM((2, W, bq), bf16),
                pltpu.SemaphoreType.DMA((nxc,)),
                pltpu.SemaphoreType.DMA((3,)),
                pltpu.SemaphoreType.DMA((noc,)),
                pltpu.SemaphoreType.DMA((2, 4)),
                pltpu.SemaphoreType.DMA(()),
            ],
            compiler_params=pltpu.CompilerParams(
                dimension_semantics=("arbitrary",), vmem_limit_bytes=100 * 1024 * 1024,
                **({"flags": flags} if flags else {})),
        )(x, k, v, A_wq, A_wo, wr, B_w_gate, B_w_up, B_w_down)
        return out.reshape(1, S, D)
    return fn


@jax.jit
def pallas_recurrent_scan__sliding_block_cached__moe_arch_mod__prompt_kernel(
        A_x, A_k_cache, A_v_cache, A_wq, A_wo, B_x, B_w_r, B_w_gate, B_w_up, B_w_down):
    return _build(order=1, dmapos=1)(A_x, A_k_cache, A_v_cache, A_wq, A_wo, B_x, B_w_r, B_w_gate, B_w_up, B_w_down)
```

```python
import jax
import jax.numpy as jnp
from jax import lax
import jax.experimental.pallas as pl
import jax.experimental.pallas.tpu as pltpu

S, D, H, DH, SK, W, F = 2048, 640, 32, 192, 2048, 512, 1536
NP = H // 2
NXC, NOC = 8, 8
LNB, FINB = 256, 128
LOG2E = 1.4426950408889634
NT = (((1,), (1,)), ((), ()))
f32, bf16 = jnp.float32, jnp.bfloat16


def _kernel(x_hbm, k_hbm, v_hbm, wq_hbm, wo_hbm, wr_hbm, wg_hbm, wu_hbm, wd_hbm, o_hbm,
            x_ref, xn_ref, g_ref, acc_ref, kp_ref, wot_ref, wg_ref, wu_ref, wd_ref,
            ob_ref, r_ref, kb_ref, vb_ref, wqb_ref, wob_ref, wr_ref,
            xsem, wsem, osem, psem, rsem):
    j = pl.program_id(0)
    slot = j % 2
    xc_rows, oc_rows = S // NXC, S // NOC

    def pcopies(p, s):
        h0 = p * 2
        c0 = pl.multiple_of(p * (2 * DH), 2 * DH)
        return [
            pltpu.make_async_copy(k_hbm.at[pl.ds(h0, 2), :, pl.ds(SK - W, W)], kb_ref.at[s], psem.at[s, 0]),
            pltpu.make_async_copy(v_hbm.at[pl.ds(h0, 2), :, pl.ds(SK - W, W)], vb_ref.at[s], psem.at[s, 1]),
            pltpu.make_async_copy(wq_hbm.at[:, pl.ds(c0, 2 * DH)], wqb_ref.at[s], psem.at[s, 2]),
            pltpu.make_async_copy(wo_hbm.at[pl.ds(c0, 2 * DH), :], wob_ref.at[s], psem.at[s, 3]),
        ]

    def xcopy(c):
        r0 = pl.multiple_of(c * xc_rows, xc_rows)
        return pltpu.make_async_copy(x_hbm.at[pl.ds(r0, xc_rows)], x_ref.at[pl.ds(r0, xc_rows)], xsem.at[c])

    def wcopies():
        return [pltpu.make_async_copy(wg_hbm, wg_ref, wsem.at[0]),
                pltpu.make_async_copy(wu_hbm, wu_ref, wsem.at[1]),
                pltpu.make_async_copy(wd_hbm, wd_ref, wsem.at[2])]

    def ocopy(c):
        r0 = pl.multiple_of(c * oc_rows, oc_rows)
        return pltpu.make_async_copy(ob_ref.at[pl.ds(r0, oc_rows)], o_hbm.at[pl.ds(r0, oc_rows)], osem.at[c])

    @pl.when(j == 0)
    def _first():
        rcopy = pltpu.make_async_copy(wr_hbm, wr_ref, rsem)
        rcopy.start()
        for c in range(NXC):
            xcopy(c).start()
        for cp in pcopies(0, 0):
            cp.start()
        acc_ref[...] = jnp.zeros_like(acc_ref)
        rcopy.wait()
        wr = wr_ref[...]

        def chunk(c, carry):
            xcopy(c).wait()
            r0 = pl.multiple_of(c * xc_rows, xc_rows)
            x = x_ref[pl.ds(r0, LNB), :].astype(f32)
            m = jnp.mean(x, axis=-1, keepdims=True)
            xc = x - m
            v = jnp.mean(xc * xc, axis=-1, keepdims=True)
            xf = xc * lax.rsqrt(v + 1e-5)
            xn = xf.astype(bf16)
            xn_ref[pl.ds(r0, LNB), :] = xn
            g_ref[pl.ds(r0, LNB), :] = xf * (0.5 + 0.5 * jnp.tanh(0.5 * xf))
            r_ref[:, pl.ds(r0, LNB)] = lax.dot_general(wr, xn, NT, preferred_element_type=f32)
            return carry
        lax.fori_loop(0, NXC, chunk, 0)
        for cp in wcopies():
            cp.start()

    @pl.when(j == 1)
    def _ffn():
        for cp in wcopies():
            cp.wait()
        r = r_ref[0:1, :]
        lane = lax.broadcasted_iota(jnp.int32, (1, S), 1)
        m1 = jnp.max(r, axis=-1, keepdims=True)
        i1 = jnp.min(jnp.where(r == m1, lane, S), axis=-1, keepdims=True)
        r2 = jnp.where(lane == i1, -jnp.inf, r)
        m2 = jnp.max(r2, axis=-1, keepdims=True)
        i2 = jnp.min(jnp.where((r2 == m2) & (lane != i1), lane, S), axis=-1, keepdims=True)
        s1 = jnp.minimum(jnp.sum(i1), S - 1)
        s2 = jnp.minimum(jnp.sum(i2), S - 1)
        rows16 = lax.broadcasted_iota(jnp.int32, (16, 1), 0)

        def pick(s):
            b0 = pl.multiple_of((s // 16) * 16, 16)
            t = xn_ref[pl.ds(b0, 16), :].astype(f32)
            return jnp.sum(jnp.where(rows16 == s - b0, t, 0.0), axis=0, keepdims=True)
        rr = lax.broadcasted_iota(jnp.int32, (8, 1), 0)
        xs = jnp.where(rr == 0, pick(s1), jnp.where(rr == 1, pick(s2), 0.0))
        xsb = xs.astype(bf16)
        gt = jnp.dot(xsb, wg_ref[...], preferred_element_type=f32)
        u = jnp.dot(xsb, wu_ref[...], preferred_element_type=f32)
        hgu = (gt * jax.nn.sigmoid(gt) * u).astype(bf16)
        y = jnp.dot(hgu, wd_ref[...], preferred_element_type=f32)
        b = xs + y * jax.nn.sigmoid(jnp.where(rr == 0, m1, m2))
        gp = b * jax.nn.sigmoid(b)
        g_ref[pl.ds(s1, 1), :] = gp[0:1, :]
        g_ref[pl.ds(s2, 1), :] = gp[1:2, :]

    for cp in pcopies(j, slot):
        cp.wait()
    k_ref, v_ref, wq_ref, wo_ref = kb_ref.at[slot], vb_ref.at[slot], wqb_ref.at[slot], wob_ref.at[slot]

    q = jnp.dot(xn_ref[...], wq_ref[...], preferred_element_type=f32)
    q = (q * (DH ** -0.5 * LOG2E)).astype(bf16)
    z64 = jnp.zeros((64, W), bf16)
    kp_ref[0] = jnp.concatenate([k_ref[0], z64], axis=0).T
    kp_ref[1] = jnp.concatenate([z64, k_ref[1]], axis=0).T
    for cp in pcopies(jnp.minimum(j + 1, NP - 1), 1 - slot):
        cp.start()
    st = [lax.dot_general(kp_ref[h], q[:, h * 128:h * 128 + 256], NT, preferred_element_type=f32)
          for h in range(2)]
    wot_ref[...] = wo_ref[...].T
    os_ = []
    for h in range(2):
        m = jnp.max(st[h], axis=0, keepdims=True)
        p = jnp.exp2(st[h] - m)
        l = jnp.sum(p, axis=0, keepdims=True)
        o = jnp.dot(v_ref[h], p.astype(bf16), preferred_element_type=f32)
        os_.append((o * (1.0 / l)).astype(bf16))
    oc = jnp.concatenate(os_, axis=0)
    acc_ref[...] += jnp.dot(wot_ref[...], oc, preferred_element_type=f32)

    @pl.when(j == NP - 1)
    def _fin():
        def chunk(c, carry):
            for u in range(oc_rows // FINB):
                r0 = pl.multiple_of(c * oc_rows + u * FINB, FINB)
                a = acc_ref[:, pl.ds(r0, FINB)].T
                ob_ref[pl.ds(r0, FINB), :] = (
                    x_ref[pl.ds(r0, FINB), :].astype(f32) + a * g_ref[pl.ds(r0, FINB), :]).astype(bf16)
            ocopy(c).start()
            return carry
        lax.fori_loop(0, NOC, chunk, 0)
        for c in range(NOC):
            ocopy(c).wait()
        for cp in pcopies(NP - 1, 1 - slot):
            cp.wait()


@jax.jit
def pallas_recurrent_scan__sliding_block_cached__moe_arch_mod__prompt_kernel(
        A_x, A_k_cache, A_v_cache, A_wq, A_wo, B_x, B_w_r, B_w_gate, B_w_up, B_w_down):
    del B_x
    x = A_x.reshape(S, D)
    k = A_k_cache.reshape(H, SK, DH).transpose(0, 2, 1)
    v = A_v_cache.reshape(H, SK, DH).transpose(0, 2, 1)
    wr = jnp.broadcast_to(B_w_r.reshape(1, D), (8, D))
    anyspec = pl.BlockSpec(memory_space=pl.ANY)
    out = pl.pallas_call(
        _kernel,
        grid=(NP,),
        in_specs=[anyspec] * 9,
        out_specs=anyspec,
        out_shape=jax.ShapeDtypeStruct((S, D), bf16),
        scratch_shapes=[
            pltpu.VMEM((S, D), bf16),
            pltpu.VMEM((S, D), bf16),
            pltpu.VMEM((S, D), f32),
            pltpu.VMEM((D, S), f32),
            pltpu.VMEM((2, W, 256), bf16),
            pltpu.VMEM((D, 2 * DH), bf16),
            pltpu.VMEM((D, F), bf16),
            pltpu.VMEM((D, F), bf16),
            pltpu.VMEM((F, D), bf16),
            pltpu.VMEM((S, D), bf16),
            pltpu.VMEM((8, S), f32),
            pltpu.VMEM((2, 2, DH, W), bf16),
            pltpu.VMEM((2, 2, DH, W), bf16),
            pltpu.VMEM((2, D, 2 * DH), bf16),
            pltpu.VMEM((2, 2 * DH, D), bf16),
            pltpu.VMEM((8, D), bf16),
            pltpu.SemaphoreType.DMA((NXC,)),
            pltpu.SemaphoreType.DMA((3,)),
            pltpu.SemaphoreType.DMA((NOC,)),
            pltpu.SemaphoreType.DMA((2, 4)),
            pltpu.SemaphoreType.DMA(()),
        ],
        compiler_params=pltpu.CompilerParams(
            dimension_semantics=("arbitrary",), vmem_limit_bytes=100 * 1024 * 1024),
    )(x, k, v, A_wq, A_wo, wr, B_w_gate, B_w_up, B_w_down)
    return out.reshape(1, S, D)
```
